```python
import os as _os
_os.environ.setdefault("JAX_PLATFORMS", "cpu")
import jax
import jax.numpy as jnp

def _softmax(x, axis=-1):
    return jax.nn.softmax(x, axis=axis)
def _gelu(x):
    return jax.nn.gelu(x, approximate=True)
def _silu(x):
    return jax.nn.silu(x)
def _sigmoid(x):
    return jax.nn.sigmoid(x)
def _layernorm(x, axis=-1, eps=1e-5):
    m = jnp.mean(x, axis=axis, keepdims=True)
    v = jnp.var(x, axis=axis, keepdims=True)
    return (x - m) / jnp.sqrt(v + eps)
def _scatter_add(tgt, idx, src, axis=0):
    return tgt.at[idx].add(src)
def _segment_sum(src, seg, n):
    return jax.ops.segment_sum(src, seg, n)
class _Rng:
    def __init__(self, key):
        self._k = key
    def _next(self):
        self._k, sub = jax.random.split(self._k)
        return sub
    def normal(self, shape):
        return jax.random.normal(self._next(), shape, dtype=jnp.bfloat16)
    def randint(self, lo, hi, shape):
        return jax.random.randint(self._next(), shape, lo, hi, dtype=jnp.int32)
    def uniform(self, shape, lo=0.0, hi=1.0):
        return jax.random.uniform(self._next(), shape, jnp.bfloat16, lo, hi)
    def permutation(self, n):
        return jax.random.permutation(self._next(), n)


kernel_name = 'parallel_sum__mha_block__swiglu_ffn__prompt'

def setup_inputs():
    _rng = _Rng(jax.random.key(int.from_bytes(__import__("os").urandom(4), "little")))
    _w = (lambda a: (lambda t: t.astype(jnp.bfloat16) if jnp.issubdtype(t.dtype, jnp.floating) else t)(jnp.asarray(a)))
    def _A_setup():
        B, S, D, H = 1, 2048, 512, 32
        return {
            "x": _w((lambda *s: _rng.normal(s) * 0.05)(B, S, D)),
            "wqkv": _w((lambda *s: _rng.normal(s) * 0.1)(D, 3 * D)),
            "wo": _w((lambda *s: _rng.normal(s) * 0.05)(D, D)),
        }
    _A_in = _A_setup()

    def _B_setup():
        B, S, D, F = 1, 2048, 512, 1792
        return {
            "x": _w((lambda *s: _rng.normal(s) * 0.05)(B, S, D)),
            "w_gate": _w((lambda *s: _rng.normal(s) * 0.05)(D, F)),
            "w_up": _w((lambda *s: _rng.normal(s) * 0.05)(D, F)),
            "w_down": _w((lambda *s: _rng.normal(s) * 0.05)(F, D)),
        }
    _B_in = _B_setup()

    return {
        "A_x": _A_in["x"],
        "A_wqkv": _A_in["wqkv"],
        "A_wo": _A_in["wo"],
        "B_x": _B_in["x"],
        "B_w_gate": _B_in["w_gate"],
        "B_w_up": _B_in["w_up"],
        "B_w_down": _B_in["w_down"],
    }

def reference(A_x, A_wqkv, A_wo, B_x, B_w_gate, B_w_up, B_w_down):
    def _A_ref(x, wqkv, wo):
        B, S, D = x.shape
        H = 32
        Dh = D // H
        qkv = (lambda x, *d: x.transpose(*d))((x @ wqkv).reshape(B, S, 3, H, Dh), 2, 0, 3, 1, 4)
        q, k, v = qkv[0], qkv[1], qkv[2]
        scores = jnp.einsum("bhqd,bhkd->bhqk", q, k) * (Dh ** -0.5)
        p = _softmax(scores, axis=-1)
        o = jnp.einsum("bhqk,bhkd->bhqd", p, v)
        return (lambda x, *d: x.transpose(*d))(o, 0, 2, 1, 3).reshape(B, S, D) @ wo

    def _B_ref(x, w_gate, w_up, w_down):
        g = _silu(x @ w_gate)
        u = x @ w_up
        return (g * u) @ w_down

    x = A_x
    xn = _layernorm(x, axis=-1)
    return x + _A_ref(xn, A_wqkv, A_wo) + _B_ref(xn, B_w_gate, B_w_up, B_w_down)
```

```python
import numpy as np
import jax
import jax.numpy as jnp
import jax.experimental.pallas as pl
import jax.experimental.pallas.tpu as pltpu

S, D, H, DH, F = 2048, 512, 32, 16, 1792
TQ = 512
RB = 512
KC = 128
HU = 4
LA = 4
FC = 256
NC = S // KC
QSCALE = float(DH ** -0.5 * np.log2(np.e))
L_SAFE = float(2.0 ** -80)
NT = (((1,), (1,)), ((), ()))
BF, F32 = jnp.bfloat16, jnp.float32


def _dot(a, b):
    return jnp.dot(a, b, preferred_element_type=F32)


def _dot_nt(a, b):
    return jax.lax.dot_general(a, b, NT, preferred_element_type=F32)


def _kernel(x_hbm, wqkv_hbm, wo_hbm, wg_hbm, wu_hbm, wd_hbm, o_ref,
            x_s, wqkv_s, wo_s, wg_s, wu_s, wd_s,
            xn_s, k_s, vt_s, q_s, ot_s, m_s, kn_s, sems):
    i = pl.program_id(0)
    e = (jax.lax.broadcasted_iota(jnp.int32, (H, D), 1) // DH
         == jax.lax.broadcasted_iota(jnp.int32, (H, D), 0)).astype(BF)

    def late_copies():
        return [pltpu.make_async_copy(src, dst, sems.at[6 + n]) for n, (src, dst) in enumerate(
            [(wo_hbm, wo_s), (wg_hbm, wg_s), (wu_hbm, wu_s), (wd_hbm, wd_s)])]

    @pl.when(i == 0)
    def _():
        xc = [pltpu.make_async_copy(x_hbm.at[pl.ds(r * RB, RB), :], x_s.at[pl.ds(r * RB, RB), :], sems.at[r])
              for r in range(S // RB)]
        wkv = pltpu.make_async_copy(wqkv_hbm.at[:, pl.ds(D, 2 * D)], wqkv_s.at[:, pl.ds(D, 2 * D)], sems.at[4])
        wq = pltpu.make_async_copy(wqkv_hbm.at[:, pl.ds(0, D)], wqkv_s.at[:, pl.ds(0, D)], sems.at[5])
        xc[0].start()
        wkv.start()
        for cp in xc[1:]:
            cp.start()
        wq.start()
        for cp in late_copies():
            cp.start()
        kn = None
        for r in range(S // RB):
            rows = pl.ds(r * RB, RB)
            xc[r].wait()
            x = x_s[rows, :].astype(F32)
            xm = x - jnp.mean(x, axis=-1, keepdims=True)
            var = jnp.mean(xm * xm, axis=-1, keepdims=True)
            xn = (xm * jax.lax.rsqrt(var + 1e-5)).astype(BF)
            xn_s[rows, :] = xn
            if r == 0:
                wkv.wait()
            kk = _dot(xn, wqkv_s[:, D:2 * D]).astype(BF)
            for g in range(D // 128):
                k_s[g, rows, :] = kk[:, g * 128:(g + 1) * 128]
            n2 = _dot_nt(e, kk * kk)
            kn = n2 if kn is None else jnp.maximum(kn, n2)
            vt = _dot(xn, wqkv_s[:, 2 * D:]).T.astype(BF)
            for h in range(H):
                vt_s[h, :, rows] = vt[h * DH:(h + 1) * DH, :]
        kn_s[...] = jnp.broadcast_to(jnp.max(kn, axis=1, keepdims=True), (H, 128))
        wq.wait()

    rows = pl.ds(pl.multiple_of(i * TQ, TQ), TQ)
    xn = xn_s[rows, :]
    q = (_dot(xn, wqkv_s[:, 0:D]) * QSCALE).astype(BF)
    for g in range(D // 128):
        q_s[g] = q[:, g * 128:(g + 1) * 128]
    m_s[...] = jnp.sqrt(_dot_nt(e, q * q) * kn_s[:, 0:1]) * 1.01
    lane_head = jax.lax.broadcasted_iota(jnp.int32, (TQ, 128), 1) // DH

    def qmask(h):
        qg = q_s[h // 8]
        return jnp.where(lane_head == h % 8, qg, jnp.zeros_like(qg))

    def put(h, ot, l):
        ot_s[pl.ds(pl.multiple_of(h * DH, DH), DH), :] = ot / l

    def fast(j, bad):
        items = [(u, c) for u in range(HU) for c in range(NC)]
        qms = [qmask(j * HU + u) for u in range(HU)]
        ms = [m_s[pl.ds(j * HU + u, 1), :] for u in range(HU)]

        def scores(u, c):
            return _dot_nt(k_s[(j * HU + u) // 8, pl.ds(c * KC, KC), :], qms[u])

        pend = [scores(*items[t]) for t in range(LA)]
        for t, (u, c) in enumerate(items):
            h = j * HU + u
            if t + LA < len(items):
                pend.append(scores(*items[t + LA]))
            p = jnp.exp2(pend.pop(0) - ms[u])
            o_c = _dot(vt_s[h, :, pl.ds(c * KC, KC)], p.astype(BF))
            l_c = jnp.sum(p.reshape(KC // 8, 8, TQ), axis=0)
            ot, l8 = (o_c, l_c) if c == 0 else (ot + o_c, l8 + l_c)
            if c == NC - 1:
                l = jnp.sum(l8, axis=0, keepdims=True)
                put(h, ot, l)
                bad = jnp.where(l >= L_SAFE, bad, 1)
        return bad

    bad = jax.lax.fori_loop(0, H // HU, fast, jnp.zeros((1, TQ), jnp.int32))

    @pl.when(jnp.max(bad) > 0)
    def _():
        def exact(h, carry):
            st = _dot_nt(k_s[h // 8], qmask(h))
            p = jnp.exp2(st - jnp.max(st, axis=0, keepdims=True))
            put(h, _dot(vt_s[h], p.astype(BF)), jnp.sum(p, axis=0, keepdims=True))
            return carry
        jax.lax.fori_loop(0, H, exact, 0)

    @pl.when(i == 0)
    def _():
        for cp in late_copies():
            cp.wait()

    acc = x_s[rows, :].astype(F32) + _dot(ot_s[...].T.astype(BF), wo_s[...])
    for c in range(F // FC):
        cs = slice(c * FC, (c + 1) * FC)
        g = _dot(xn, wg_s[:, cs])
        u = _dot(xn, wu_s[:, cs])
        acc = acc + _dot((g * jax.nn.sigmoid(g) * u).astype(BF), wd_s[cs, :])
    o_ref[...] = acc.astype(o_ref.dtype)


@jax.jit
def pallas_parallel_sum__mha_block__swiglu_ffn__prompt_kernel(
    A_x: jax.Array,
    A_wqkv: jax.Array,
    A_wo: jax.Array,
    B_x: jax.Array,
    B_w_gate: jax.Array,
    B_w_up: jax.Array,
    B_w_down: jax.Array,
):
    del B_x
    out = pl.pallas_call(
        _kernel,
        grid=(S // TQ,),
        in_specs=[pl.BlockSpec(memory_space=pl.ANY)] * 6,
        out_specs=pl.BlockSpec((TQ, D), lambda i: (i, 0)),
        out_shape=jax.ShapeDtypeStruct((S, D), A_x.dtype),
        scratch_shapes=[
            pltpu.VMEM((S, D), BF), pltpu.VMEM((D, 3 * D), BF), pltpu.VMEM((D, D), BF),
            pltpu.VMEM((D, F), BF), pltpu.VMEM((D, F), BF), pltpu.VMEM((F, D), BF),
            pltpu.VMEM((S, D), BF), pltpu.VMEM((D // 128, S, 128), BF), pltpu.VMEM((H, DH, S), BF),
            pltpu.VMEM((D // 128, TQ, 128), BF), pltpu.VMEM((D, TQ), F32), pltpu.VMEM((H, TQ), F32),
            pltpu.VMEM((H, 128), F32), pltpu.SemaphoreType.DMA((10,)),
        ],
        compiler_params=pltpu.CompilerParams(
            dimension_semantics=("arbitrary",), vmem_limit_bytes=64 * 2**20),
    )(A_x.reshape(S, D), A_wqkv, A_wo, B_w_gate, B_w_up, B_w_down)
    return out.reshape(1, S, D)
```

```python
import numpy as np
import jax
import jax.numpy as jnp
import jax.experimental.pallas as pl
import jax.experimental.pallas.tpu as pltpu

S, D, H, DH, F = 2048, 512, 32, 16, 1792
TQ = 512
RB = 512
KC = 128
HU = 8
LA = 5
QN = 256
FC = 256
NC = S // KC
QSCALE = float(DH ** -0.5 * np.log2(np.e))
L_SAFE = float(2.0 ** -80)
L_MAX = float(2 * S)
NT = (((1,), (1,)), ((), ()))
BF, F32 = jnp.bfloat16, jnp.float32


def _dot(a, b):
    return jnp.dot(a, b, preferred_element_type=F32)


def _dot_nt(a, b):
    return jax.lax.dot_general(a, b, NT, preferred_element_type=F32)


def _kernel(x_hbm, wqkv_hbm, wo_hbm, wg_hbm, wu_hbm, wd_hbm, o_ref,
            x_s, wqkv_s, wo_s, wg_s, wu_s, wd_s,
            xn_s, k_s, vt_s, q_s, ot_s, m_s, kn_s, sems):
    i = pl.program_id(0)
    e = (jax.lax.broadcasted_iota(jnp.int32, (H, D), 1) // DH
         == jax.lax.broadcasted_iota(jnp.int32, (H, D), 0)).astype(BF)

    def late_copies():
        return [pltpu.make_async_copy(src, dst, sems.at[6 + n]) for n, (src, dst) in enumerate(
            [(wo_hbm, wo_s), (wg_hbm, wg_s), (wu_hbm, wu_s), (wd_hbm, wd_s)])]

    @pl.when(i == 0)
    def _():
        xc = [pltpu.make_async_copy(x_hbm.at[pl.ds(r * RB, RB), :], x_s.at[pl.ds(r * RB, RB), :], sems.at[r])
              for r in range(S // RB)]
        wkv = pltpu.make_async_copy(wqkv_hbm.at[:, pl.ds(D, 2 * D)], wqkv_s.at[:, pl.ds(D, 2 * D)], sems.at[4])
        wq = pltpu.make_async_copy(wqkv_hbm.at[:, pl.ds(0, D)], wqkv_s.at[:, pl.ds(0, D)], sems.at[5])
        xc[0].start()
        wkv.start()
        for cp in xc[1:]:
            cp.start()
        wq.start()
        for cp in late_copies():
            cp.start()
        kn = None
        for r in range(S // RB):
            rows = pl.ds(r * RB, RB)
            xc[r].wait()
            x = x_s[rows, :].astype(F32)
            xm = x - jnp.mean(x, axis=-1, keepdims=True)
            var = jnp.mean(xm * xm, axis=-1, keepdims=True)
            xn = (xm * jax.lax.rsqrt(var + 1e-5)).astype(BF)
            xn_s[rows, :] = xn
            if r == 0:
                wkv.wait()
            kk = _dot(xn, wqkv_s[:, D:2 * D]).astype(BF)
            for g in range(D // 128):
                k_s[g, rows, :] = kk[:, g * 128:(g + 1) * 128]
            n2 = _dot_nt(e, kk * kk)
            kn = n2 if kn is None else jnp.maximum(kn, n2)
            vt = _dot(xn, wqkv_s[:, 2 * D:]).T.astype(BF)
            for h in range(H):
                vt_s[h, :, rows] = vt[h * DH:(h + 1) * DH, :]
        kn_s[...] = jnp.broadcast_to(jnp.max(kn, axis=1, keepdims=True), (H, 128))
        wq.wait()

    rows = pl.ds(pl.multiple_of(i * TQ, TQ), TQ)
    xn = xn_s[rows, :]
    q = (_dot(xn, wqkv_s[:, 0:D]) * QSCALE).astype(BF)
    for g in range(D // 128):
        q_s[g] = q[:, g * 128:(g + 1) * 128]
    m_s[...] = jnp.sqrt(_dot_nt(e, q * q) * kn_s[:, 0:1]) * 1.01
    lane_head = jax.lax.broadcasted_iota(jnp.int32, (TQ, 128), 1) // DH

    def qmask(h):
        qg = q_s[h // 8]
        return jnp.where(lane_head == h % 8, qg, jnp.zeros_like(qg))

    def put(h, ot, l):
        ot_s[pl.ds(pl.multiple_of(h * DH, DH), DH), :] = ot / l

    def fast(j, bad):
        NQ = TQ // QN
        items = [(u, c, n) for u in range(HU) for c in range(NC) for n in range(NQ)]
        qms = [qmask(j * HU + u) for u in range(HU)]
        ms = [m_s[pl.ds(j * HU + u, 1), :] for u in range(HU)]

        def scores(u, c, n):
            return _dot_nt(k_s[(j * HU + u) // 8, pl.ds(c * KC, KC), :], qms[u][n * QN:(n + 1) * QN])

        pend = [scores(*items[t]) for t in range(LA)]
        ot, l8 = [None] * NQ, [None] * NQ
        for t, (u, c, n) in enumerate(items):
            h = j * HU + u
            if t + LA < len(items):
                pend.append(scores(*items[t + LA]))
            p = jnp.exp2(pend.pop(0) - ms[u][:, n * QN:(n + 1) * QN])
            o_c = _dot(vt_s[h, :, pl.ds(c * KC, KC)], p.astype(BF))
            l_c = jnp.sum(p.reshape(KC // 8, 8, QN), axis=0)
            ot[n], l8[n] = (o_c, l_c) if c == 0 else (ot[n] + o_c, l8[n] + l_c)
            if c == NC - 1 and n == NQ - 1:
                l = jnp.sum(jnp.concatenate(l8, axis=1), axis=0, keepdims=True)
                put(h, jnp.concatenate(ot, axis=1), l)
                bad = jnp.where((l >= L_SAFE) & (l <= L_MAX), bad, 1)
        return bad

    bad = jax.lax.fori_loop(0, H // HU, fast, jnp.zeros((1, TQ), jnp.int32))

    @pl.when(jnp.max(bad) > 0)
    def _():
        def exact(h, carry):
            st = _dot_nt(k_s[h // 8], qmask(h))
            p = jnp.exp2(st - jnp.max(st, axis=0, keepdims=True))
            put(h, _dot(vt_s[h], p.astype(BF)), jnp.sum(p, axis=0, keepdims=True))
            return carry
        jax.lax.fori_loop(0, H, exact, 0)

    @pl.when(i == 0)
    def _():
        for cp in late_copies():
            cp.wait()

    acc = x_s[rows, :].astype(F32) + _dot(ot_s[...].T.astype(BF), wo_s[...])
    for c in range(F // FC):
        cs = slice(c * FC, (c + 1) * FC)
        g = _dot(xn, wg_s[:, cs])
        u = _dot(xn, wu_s[:, cs])
        acc = acc + _dot((g * jax.nn.sigmoid(g) * u).astype(BF), wd_s[cs, :])
    o_ref[...] = acc.astype(o_ref.dtype)


@jax.jit
def pallas_parallel_sum__mha_block__swiglu_ffn__prompt_kernel(
    A_x: jax.Array,
    A_wqkv: jax.Array,
    A_wo: jax.Array,
    B_x: jax.Array,
    B_w_gate: jax.Array,
    B_w_up: jax.Array,
    B_w_down: jax.Array,
):
    del B_x
    out = pl.pallas_call(
        _kernel,
        grid=(S // TQ,),
        in_specs=[pl.BlockSpec(memory_space=pl.ANY)] * 6,
        out_specs=pl.BlockSpec((TQ, D), lambda i: (i, 0)),
        out_shape=jax.ShapeDtypeStruct((S, D), A_x.dtype),
        scratch_shapes=[
            pltpu.VMEM((S, D), BF), pltpu.VMEM((D, 3 * D), BF), pltpu.VMEM((D, D), BF),
            pltpu.VMEM((D, F), BF), pltpu.VMEM((D, F), BF), pltpu.VMEM((F, D), BF),
            pltpu.VMEM((S, D), BF), pltpu.VMEM((D // 128, S, 128), BF), pltpu.VMEM((H, DH, S), BF),
            pltpu.VMEM((D // 128, TQ, 128), BF), pltpu.VMEM((D, TQ), F32), pltpu.VMEM((H, TQ), F32),
            pltpu.VMEM((H, 128), F32), pltpu.SemaphoreType.DMA((10,)),
        ],
        compiler_params=pltpu.CompilerParams(
            dimension_semantics=("arbitrary",), vmem_limit_bytes=64 * 2**20),
    )(A_x.reshape(S, D), A_wqkv, A_wo, B_w_gate, B_w_up, B_w_down)
    return out.reshape(1, S, D)
```
